```python
import os as _os
_os.environ.setdefault("JAX_PLATFORMS", "cpu")
import jax
import jax.numpy as jnp

def _softmax(x, axis=-1):
    return jax.nn.softmax(x, axis=axis)
def _gelu(x):
    return jax.nn.gelu(x, approximate=True)
def _silu(x):
    return jax.nn.silu(x)
def _sigmoid(x):
    return jax.nn.sigmoid(x)
def _layernorm(x, axis=-1, eps=1e-5):
    m = jnp.mean(x, axis=axis, keepdims=True)
    v = jnp.var(x, axis=axis, keepdims=True)
    return (x - m) / jnp.sqrt(v + eps)
def _scatter_add(tgt, idx, src, axis=0):
    return tgt.at[idx].add(src)
def _segment_sum(src, seg, n):
    return jax.ops.segment_sum(src, seg, n)
class _Rng:
    def __init__(self, key):
        self._k = key
    def _next(self):
        self._k, sub = jax.random.split(self._k)
        return sub
    def normal(self, shape):
        return jax.random.normal(self._next(), shape, dtype=jnp.bfloat16)
    def randint(self, lo, hi, shape):
        return jax.random.randint(self._next(), shape, lo, hi, dtype=jnp.int32)
    def uniform(self, shape, lo=0.0, hi=1.0):
        return jax.random.uniform(self._next(), shape, jnp.bfloat16, lo, hi)
    def permutation(self, n):
        return jax.random.permutation(self._next(), n)


kernel_name = 'concat_heads__sliding_block_cached__compressed_kv_cla__decode'

def setup_inputs():
    _rng = _Rng(jax.random.key(int.from_bytes(__import__("os").urandom(4), "little")))
    _w = (lambda a: (lambda t: t.astype(jnp.bfloat16) if jnp.issubdtype(t.dtype, jnp.floating) else t)(jnp.asarray(a)))
    def _A_setup():
        B, Sq, D = 1, 1, 512
        Hq, Hkv, Sk, Dh = 32, 32, 4096, 128
        assert Hq % Hkv == 0, (Hq, Hkv)
        return {
            "x": _w((lambda *s: _rng.normal(s) * 0.8)(B, Sq, D)),
            "k_cache": _w((lambda *s: _rng.normal(s) * 0.8)(B, Hkv, Sk, Dh)),
            "v_cache": _w((lambda *s: _rng.normal(s) * 0.05)(B, Hkv, Sk, Dh)),
            "wq": _w((lambda *s: _rng.normal(s) * 0.8)(D, Hq * Dh) * (D ** -0.5)),
            "wo": _w((lambda *s: _rng.normal(s) * 0.05)(Hq * Dh, D) * ((Hq * Dh) ** -0.5)),
        }
    _A_in = _A_setup()

    def _B_setup():
        B, H, Sq, Sk, D, M = 1, 32, 1, 4096, 128, 512
        Dc = 4 * D
        return {
            "x": _w((lambda *s: _rng.normal(s) * 1.6)(B, Sq, M)),
            "c_kv": _w((lambda *s: _rng.normal(s) * 0.1)(B, Sk, Dc)),
            "w_q": _w((lambda *s: _rng.normal(s) * 1.6)(M, H, D) * (M ** -0.5)),
            "w_uk": _w((lambda *s: _rng.normal(s) * 1.6)(Dc, H, D) * (Dc ** -0.5)),
            "w_uv": _w((lambda *s: _rng.normal(s) * 0.1)(Dc, H, D) * (Dc ** -0.5)),
            "w_o": _w((lambda *s: _rng.normal(s) * 0.1)(H, D, M) * ((H * D) ** -0.5)),
        }
    _B_in = _B_setup()

    return {
        "A_x": _A_in["x"],
        "A_k_cache": _A_in["k_cache"],
        "A_v_cache": _A_in["v_cache"],
        "A_wq": _A_in["wq"],
        "A_wo": _A_in["wo"],
        "B_x": _B_in["x"],
        "B_c_kv": _B_in["c_kv"],
        "B_w_q": _B_in["w_q"],
        "B_w_uk": _B_in["w_uk"],
        "B_w_uv": _B_in["w_uv"],
        "B_w_o": _B_in["w_o"],
    }

def reference(A_x, A_k_cache, A_v_cache, A_wq, A_wo, B_x, B_c_kv, B_w_q, B_w_uk, B_w_uv, B_w_o):
    def _A_ref(x, k_cache, v_cache, wq, wo):
        B, Sq, D = x.shape
        Hq, Dh = 32, 128
        Hkv, Sk = k_cache.shape[1], k_cache.shape[2]
        W = min(4096, max(256, Sk // 4))
        rep = Hq // Hkv
        q = (lambda x, *d: x.transpose(*d))((x @ wq).reshape(B, Sq, Hq, Dh), 0, 2, 1, 3)
        k = jnp.repeat(k_cache[:, :, Sk - W:, :], rep, axis=1)
        v = jnp.repeat(v_cache[:, :, Sk - W:, :], rep, axis=1)
        scores = jnp.einsum("bhqd,bhkd->bhqk", q, k) * (Dh ** -0.5)
        p = _softmax(scores, axis=-1)
        o = jnp.einsum("bhqk,bhkd->bhqd", p, v)
        return (lambda x, *d: x.transpose(*d))(o, 0, 2, 1, 3).reshape(B, Sq, Hq * Dh) @ wo

    def _B_ref(x, c_kv, w_q, w_uk, w_uv, w_o):
        B, Sq, M = x.shape[0], x.shape[1], x.shape[2]
        Sk = c_kv.shape[1]
        H, D = w_q.shape[1], w_q.shape[2]
        q = jnp.einsum("bqm,mhd->bhqd", x, w_q)
        k = jnp.einsum("bkc,chd->bhkd", c_kv, w_uk)
        v = jnp.einsum("bkc,chd->bhkd", c_kv, w_uv)
        scores = jnp.einsum("bhqd,bhkd->bhqk", q, k) * (D ** -0.5)
        off = Sk - Sq
        qi = jnp.arange(Sq)[:, None]
        kj = jnp.arange(Sk)[None, :]
        cmask = kj <= (qi + off)
        scores = jnp.where(cmask[None, None], scores, -1e9)
        p = _softmax(scores, axis=-1)
        ctx = jnp.einsum("bhqk,bhkd->bhqd", p, v)
        return jnp.einsum("bhqd,hdm->bqm", ctx, w_o)

    a = _A_ref(A_x, A_k_cache, A_v_cache, A_wq, A_wo)
    b = _B_ref(B_x, B_c_kv, B_w_q, B_w_uk, B_w_uv, B_w_o)
    return jnp.concatenate([a, b], axis=-1)
```

```python
import functools
import jax
import jax.numpy as jnp
from jax import lax
from jax.experimental import pallas as pl
from jax.experimental.pallas import tpu as pltpu

BF = jnp.bfloat16
F32 = jnp.float32
H = 32
DH = 128
DM = 512
NT = (((1,), (1,)), ((), ()))


def _dot(a, b):
    return jnp.dot(a, b, preferred_element_type=F32)


def _dot_nt(a, b):
    return lax.dot_general(a, b, NT, preferred_element_type=F32)


def make(wo_chunks=(23, 8, 1), x_prio=0, compute=True, scopes=False, unroll_j=1, unroll_h=1):
    assert sum(wo_chunks) == H
    import contextlib
    scope = (lambda n: jax.named_scope(n)) if scopes else (lambda n: contextlib.nullcontext())

    def kernel(ax_h, kc_h, vc_h, wq_h, wo_h, bx_h, ckv_h, bwq_h, wuk_h, wuv_h, bwo_h, o_ref,
               ax_b, bx_b, k_b, v_b, wq_b, wo_b, ckv_b, bwq_b, wuk_b, wuv_b, bwo_b,
               sb_ref, qa_ref, pa_ref, la_ref, oa_ref, cb_ref, sems):
        sk = kc_h.shape[2]
        w = k_b.shape[1]
        cp = lambda s, d, i: pltpu.make_async_copy(s, d, sems.at[i])
        c_bwq = cp(bwq_h, bwq_b, 0)
        c_bx = cp(bx_h, bx_b, 1)
        c_ax = cp(ax_h, ax_b, 2)
        c_wuk = cp(wuk_h, wuk_b, 3)
        c_ckv = cp(ckv_h.at[0], ckv_b, 4)
        c_wuv = cp(wuv_h, wuv_b, 5)
        c_wq = cp(wq_h, wq_b, 6)
        c_k = cp(kc_h.at[0, :, pl.ds(sk - w, w), :], k_b, 7)
        c_v = cp(vc_h.at[0, :, pl.ds(sk - w, w), :], v_b, 8)
        c_bwo = cp(bwo_h, bwo_b, 9)
        c_wo = []
        h0 = 0
        for i, n in enumerate(wo_chunks):
            c_wo.append(cp(wo_h.at[pl.ds(h0 * DH, n * DH)], wo_b.at[pl.ds(h0 * DH, n * DH)], 10 + i))
            h0 += n
        c_bwq.start()
        c_bx.start(priority=x_prio)
        c_ax.start(priority=x_prio)
        for c in (c_wuk, c_ckv, c_wuv, c_wq, c_k, c_v, c_bwo, *c_wo):
            c.start()

        if not compute:
            for c in (c_bwq, c_bx, c_ax, c_wuk, c_ckv, c_wuv, c_wq, c_k, c_v, c_bwo, *c_wo):
                c.wait()
            o_ref[...] = jnp.zeros(o_ref.shape, o_ref.dtype)
            return

        row = lax.broadcasted_iota(jnp.int32, (128, 128), 0)
        lane = lax.broadcasted_iota(jnp.int32, (128, 128), 1)

        def diag_mask():
            return (row & (H - 1)) == (lane & (H - 1))

        def w_tile(ref, b, j):
            return ref[pl.ds(b * 128 + j * 4, 4)].reshape(128, 128)

        def contract_lead(a, w_ref):
            def body(j, acc):
                et = (row - (lane >> 5) == 4 * j).astype(BF)
                s = jnp.where(diag_mask(), _dot(a, et), 0.0).astype(BF)
                for b in range(4):
                    acc = acc + _dot(s[b * H:(b + 1) * H], w_tile(w_ref, b, j))
                return acc
            return lax.fori_loop(0, 32, body, jnp.zeros((H, DH), F32), unroll=unroll_j)

        with scope("w_bwq"):
            c_bx.wait()
            c_bwq.wait()
        with scope("c_bwq"):
            xb = bx_b[0].astype(F32)
            a = jnp.concatenate(
                [jnp.broadcast_to(xb[:, b * 128:(b + 1) * 128], (H, 128)) for b in range(4)], axis=0).astype(BF)
            qb = contract_lead(a, bwq_b).astype(BF)

        with scope("w_wuk"):
            c_wuk.wait()
        with scope("c_wuk"):
            def uk_body(j, acc):
                r = jnp.concatenate([_dot_nt(qb, w_tile(wuk_b, b, j)) for b in range(4)], axis=0)
                r = jnp.where(diag_mask(), r, 0.0).astype(BF)
                e = (lane - (row >> 5) == 4 * j).astype(BF)
                return acc + _dot(r, e)
            qabs = lax.fori_loop(0, 32, uk_body, jnp.zeros((128, 128), F32), unroll=unroll_j)
            qabs = jnp.concatenate([qabs[b * H:(b + 1) * H] for b in range(4)], axis=1).astype(BF)

        with scope("w_ckv"):
            c_ckv.wait()
        with scope("c_ckv"):
            nck = sb_ref.shape[0]
            ck = sb_ref.shape[2]
            scale = DH ** -0.5

            def s_body(i, m):
                c = ckv_b[pl.ds(pl.multiple_of(i * ck, ck), ck), :]
                s = _dot_nt(qabs, c) * scale
                sb_ref[i] = s
                return jnp.maximum(m, s)
            m = lax.fori_loop(0, nck, s_body, jnp.full((H, ck), -jnp.inf, F32))
            m = jnp.max(m, axis=1, keepdims=True)

            def pv_body(i, carry):
                l, acc = carry
                p = jnp.exp(sb_ref[i] - m)
                c = ckv_b[pl.ds(pl.multiple_of(i * ck, ck), ck), :]
                return l + p, acc + _dot(p.astype(BF), c)
            l, clat = lax.fori_loop(0, nck, pv_body, (jnp.zeros((H, ck), F32), jnp.zeros((H, DM), F32)))
            clat = clat / jnp.sum(l, axis=1, keepdims=True)
            clat = jnp.concatenate([clat[:, b * 128:(b + 1) * 128] for b in range(4)], axis=0).astype(BF)

        with scope("w_wuv"):
            c_wuv.wait()
        with scope("c_wuv"):
            ctx = contract_lead(clat, wuv_b)
            for h in range(H):
                cb_ref[h] = jnp.broadcast_to(ctx[h:h + 1, :], (8, DH))

        with scope("w_wq"):
            c_ax.wait()
            c_wq.wait()
        with scope("c_wq"):
            xa = jnp.broadcast_to(ax_b[0].astype(F32), (8, DM)).astype(BF)

            def q_body(i, _):
                q = _dot(xa, wq_b[:, pl.ds(pl.multiple_of(i * 512, 512), 512)])
                for t in range(4):
                    qa_ref[i * 4 + t] = q[:, t * DH:(t + 1) * DH]
                return 0
            lax.fori_loop(0, H // 4, q_body, 0)

        with scope("w_k"):
            c_k.wait()
        with scope("c_k"):
            def k_body(h, _):
                s = _dot_nt(qa_ref[h].astype(BF), k_b[h]) * scale
                p = jnp.exp(s - jnp.max(s, axis=1, keepdims=True))
                pa_ref[h] = p
                la_ref[h] = jnp.broadcast_to(jnp.sum(p, axis=1, keepdims=True), (8, DH))
                return 0
            lax.fori_loop(0, H, k_body, 0, unroll=unroll_h)

        with scope("w_v"):
            c_v.wait()
        with scope("c_v"):
            def v_body(h, _):
                oa_ref[h] = _dot(pa_ref[h].astype(BF), v_b[h]) / la_ref[h]
                return 0
            lax.fori_loop(0, H, v_body, 0, unroll=unroll_h)

        with scope("w_bwo"):
            c_bwo.wait()
        with scope("c_bwo"):
            def bo_body(h, acc):
                return acc + _dot(cb_ref[h].astype(BF), bwo_b[h])
            ob = lax.fori_loop(0, H, bo_body, jnp.zeros((8, DM), F32), unroll=unroll_h)
            o_ref[0, :, DM:2 * DM] = ob[0:1].astype(o_ref.dtype)

        def ao_body(h, acc):
            return acc + _dot(oa_ref[h].astype(BF), wo_b[pl.ds(pl.multiple_of(h * DH, DH), DH), :])
        acc = jnp.zeros((8, DM), F32)
        h0 = 0
        for i, n in enumerate(wo_chunks):
            with scope(f"w_wo{i}"):
                c_wo[i].wait()
            with scope(f"c_wo{i}"):
                if n <= 8:
                    for h in range(h0, h0 + n):
                        acc = acc + _dot(oa_ref[h].astype(BF), wo_b[h * DH:(h + 1) * DH, :])
                else:
                    acc = lax.fori_loop(h0, h0 + n, ao_body, acc, unroll=unroll_h)
            h0 += n
        o_ref[0, :, 0:DM] = acc[0:1].astype(o_ref.dtype)

    def fn(A_x, A_k_cache, A_v_cache, A_wq, A_wo, B_x, B_c_kv, B_w_q, B_w_uk, B_w_uv, B_w_o):
        sk = A_k_cache.shape[2]
        w = min(4096, max(256, sk // 4))
        skb = B_c_kv.shape[1]
        ck = 512
        hbm = pl.BlockSpec(memory_space=pltpu.HBM)
        V = pltpu.VMEM
        return pl.pallas_call(
            kernel,
            out_shape=jax.ShapeDtypeStruct((1, 1, 2 * DM), BF),
            in_specs=[hbm] * 11,
            out_specs=pl.BlockSpec(memory_space=pltpu.VMEM),
            scratch_shapes=[
                V((1, 1, DM), BF), V((1, 1, DM), BF),
                V((H, w, DH), BF), V((H, w, DH), BF),
                V((DM, H * DH), BF), V((H * DH, DM), BF),
                V((skb, DM), BF), V((DM, H, DH), BF), V((DM, H, DH), BF), V((DM, H, DH), BF),
                V((H, DH, DM), BF),
                V((skb // ck, H, ck), F32),
                V((H, 8, DH), F32), V((H, 8, w), F32), V((H, 8, DH), F32), V((H, 8, DH), F32),
                V((H, 8, DH), F32),
                pltpu.SemaphoreType.DMA((10 + len(wo_chunks),)),
            ],
            compiler_params=pltpu.CompilerParams(vmem_limit_bytes=64 * 1024 * 1024),
        )(A_x, A_k_cache, A_v_cache, A_wq, A_wo, B_x, B_c_kv, B_w_q, B_w_uk, B_w_uv, B_w_o)
    return fn


@jax.jit
def pallas_concat_heads__sliding_block_cached__compressed_kv_cla__decode_kernel(
    A_x, A_k_cache, A_v_cache, A_wq, A_wo, B_x, B_c_kv, B_w_q, B_w_uk, B_w_uv, B_w_o,
):
    return make(unroll_j=4, unroll_h=4, wo_chunks=(20, 8, 3, 1))(
        A_x, A_k_cache, A_v_cache, A_wq, A_wo, B_x, B_c_kv, B_w_q, B_w_uk, B_w_uv, B_w_o)
```

```python
import contextlib
import jax
import jax.numpy as jnp
from jax import lax
from jax.experimental import pallas as pl
from jax.experimental.pallas import tpu as pltpu

BF = jnp.bfloat16
F32 = jnp.float32
H = 32
DH = 128
DM = 512
NT = (((1,), (1,)), ((), ()))
STEPS = 8


def _dot(a, b):
    return jnp.dot(a, b, preferred_element_type=F32)


def _dot_nt(a, b):
    return lax.dot_general(a, b, NT, preferred_element_type=F32)


def make(q=24, kv_rows=(208, 208, 208, 208, 192), wq_cols=(1536, 1536, 1024), lead_n=6, row_n=48,
         small=(16,) * 24, n_vpu=2, vpu_groups=(8, 4, 2, 1, 1), wo_early=8, batch=(4, 4, 4, 4, 3, 3, 2, 2, 1),
         compute=True, scopes=False):
    scope = (lambda n: jax.named_scope(n)) if scopes else (lambda n: contextlib.nullcontext())
    big_rows = H * DH - sum(small)
    sizes = [row_n] * (big_rows // row_n)
    rem = big_rows - sum(sizes)
    if rem:
        if rem + row_n <= 64:
            sizes[0:1] = [(rem + row_n) // 2 // 8 * 8, rem + row_n - (rem + row_n) // 2 // 8 * 8]
        else:
            sizes.insert(0, rem)
    n_lo = (len(sizes) + len(small)) // 2
    sizes = sizes + list(small)
    wo_chunks = [(sum(sizes[:i]), n) for i, n in enumerate(sizes)]
    arrival = [i if i < n_lo else i - n_lo + q for i in range(len(sizes))]
    vpu_start = (H - n_vpu) * DH

    def chunks_of(r0, r1):
        return [i for i, (s, n) in enumerate(wo_chunks) if s < r1 and s + n > r0]
    mxu_heads = sorted(range(H - n_vpu), key=lambda h: max(arrival[i] for i in chunks_of(h * DH, (h + 1) * DH)))

    def kernel(ax_h, kc_h, vc_h, wq_h, wo_h, bx_h, ckv_h, bwq_h, wuk_h, wuv_h, bwo_h, o_ref,
               ax_b, bx_b, k_b, v_b, wq_b, wo_b, ckv_b, bwq_b, wuk_b, wuv_b, bwo_b,
               sb_ref, qa_ref, pa_ref, la_ref, oa_ref, cb_ref, ot_ref):
        sk = kc_h.shape[2]
        w = k_b.shape[1]
        scale = DH ** -0.5

        def main(sems, wo_sems):
            def start(src, dst, sem, priority):
                pltpu.make_async_copy(src, dst, sem).start(priority=priority)

            def start_rows(src, dst, sem, r0, n, align):
                half = dst.shape[0] // 2
                for base, priority in ((half, 1), (0, 0)):
                    r = base + r0
                    r = pl.ds(r if isinstance(r, int) else pl.multiple_of(r, align), n)
                    start(src.at[r], dst.at[r], sem[priority] if isinstance(sem, tuple) else sem, priority)

            def row_stream(src, dst, sem, n, align):
                half = dst.shape[0] // 2
                per = half // n // STEPS

                def step(t):
                    for i in range(per):
                        start_rows(src, dst, sem, (t * per + i) * n, n, align)

                def rest():
                    for r0 in range(per * STEPS * n, half, n):
                        start_rows(src, dst, sem, r0, min(n, half - r0), align)
                return step, rest

            def wq_step(g):
                c0 = 0
                for n in wq_cols:
                    for base, priority in ((DM // 2, 1), (0, 0)):
                        r = pl.ds(pl.multiple_of(base + g * 16, 16), 16)
                        start(wq_h.at[r, pl.ds(c0, n)], wq_b.at[r, pl.ds(c0, n)], sems.at[4], priority)
                    c0 += n

            def cache_step(src, dst, sem, h):
                r0 = 0
                for n in kv_rows:
                    for base, priority in ((H // 2, 1), (0, 0)):
                        start(src.at[0, base + h, pl.ds(sk - w + r0, n), :],
                              dst.at[base + h, pl.ds(r0, n), :], sem, priority)
                    r0 += n

            def wo_copy(i):
                r = pl.ds(*wo_chunks[i])
                return pltpu.make_async_copy(wo_h.at[r], wo_b.at[r], wo_sems.at[i])

            def wo_pairs(j0, j1):
                for j in range(j0, j1):
                    if n_lo + j < len(wo_chunks):
                        wo_copy(n_lo + j).start(priority=1)
                    if j < n_lo:
                        wo_copy(j).start(priority=0)

            def wait_all(buf, sem):
                pltpu.make_async_copy(buf, buf, sem).wait()

            def stage(body, init, issue, rest=None):
                def step(t, carry):
                    issue(t)
                    return body(t, carry) if compute and body is not None else carry
                out = lax.fori_loop(0, STEPS, step, init)
                if rest is not None:
                    rest()
                return out

            c_bx = pltpu.make_async_copy(bx_h, bx_b, sems.at[8])
            c_ax = pltpu.make_async_copy(ax_h, ax_b, sems.at[9])

            first = [(r0, min(lead_n, DM - r0)) for r0 in range(0, DM, lead_n)]
            n0 = (len(first) - q) // 2
            lo, hi = first[:n0], first[n0:]
            for j, (r0, n) in enumerate(hi):
                start(bwq_h.at[pl.ds(r0, n)], bwq_b.at[pl.ds(r0, n)], sems.at[0], 1)
                if j == 0:
                    c_bx.start()
                    c_ax.start()
                if q <= j < q + n0:
                    r0, n = lo[j - q]
                    start(bwq_h.at[pl.ds(r0, n)], bwq_b.at[pl.ds(r0, n)], sems.at[0], 0)
            stage(None, None, *row_stream(wuk_h, wuk_b, sems.at[1], lead_n, 1))

            row = lax.broadcasted_iota(jnp.int32, (128, 128), 0)
            lane = lax.broadcasted_iota(jnp.int32, (128, 128), 1)

            def diag_mask():
                return (row & (H - 1)) == (lane & (H - 1))

            def w_tile(ref, b, j):
                return ref[pl.ds(b * 128 + j * 4, 4)].reshape(128, 128)

            def contract_lead(a, w_ref, *issue):
                def body(t, acc):
                    for u in range(4):
                        j = t * 4 + u
                        et = (row - (lane >> 5) == 4 * j).astype(BF)
                        s = jnp.where(diag_mask(), _dot(a, et), 0.0).astype(BF)
                        for b in range(4):
                            acc = acc + _dot(s[b * H:(b + 1) * H], w_tile(w_ref, b, j))
                    return acc
                return stage(body, jnp.zeros((H, DH), F32), *issue)

            with scope("w_bwq"):
                c_bx.wait()
                wait_all(bwq_b, sems.at[0])
            with scope("c_bwq"):
                xb = bx_b[0].astype(F32)
                a = jnp.concatenate(
                    [jnp.broadcast_to(xb[:, b * 128:(b + 1) * 128], (H, 128)) for b in range(4)], axis=0).astype(BF)
                qb = contract_lead(a, bwq_b, *row_stream(ckv_h.at[0], ckv_b, sems.at[2], row_n, 8)).astype(BF)

            with scope("w_wuk"):
                wait_all(wuk_b, sems.at[1])
            with scope("c_wuk"):
                def uk_body(t, acc):
                    for u in range(4):
                        j = t * 4 + u
                        r = jnp.concatenate([_dot_nt(qb, w_tile(wuk_b, b, j)) for b in range(4)], axis=0)
                        r = jnp.where(diag_mask(), r, 0.0).astype(BF)
                        e = (lane - (row >> 5) == 4 * j).astype(BF)
                        acc = acc + _dot(r, e)
                    return acc
                qabs = stage(uk_body, jnp.zeros((128, 128), F32), *row_stream(wuv_h, wuv_b, sems.at[3], lead_n, 1))
                qabs = jnp.concatenate([qabs[b * H:(b + 1) * H] for b in range(4)], axis=1).astype(BF)

            with scope("w_ckv"):
                wait_all(ckv_b, sems.at[2])
            with scope("c_ckv"):
                ck = sb_ref.shape[2]

                def s_body(i, m):
                    c = ckv_b[pl.ds(pl.multiple_of(i * ck, ck), ck), :]
                    s = _dot_nt(qabs, c) * scale
                    sb_ref[i] = s
                    return jnp.maximum(m, s)
                m = stage(s_body, jnp.full((H, ck), -jnp.inf, F32), wq_step)
                m = jnp.max(m, axis=1, keepdims=True)

                def pv_body(i, carry):
                    l, acc = carry
                    p = jnp.exp(sb_ref[i] - m)
                    c = ckv_b[pl.ds(pl.multiple_of(i * ck, ck), ck), :]
                    return l + p, acc + _dot(p.astype(BF), c)
                l, clat = stage(pv_body, (jnp.zeros((H, ck), F32), jnp.zeros((H, DM), F32)),
                                lambda t: wq_step(STEPS + t))
                clat = clat / jnp.sum(l, axis=1, keepdims=True)
                clat = jnp.concatenate([clat[:, b * 128:(b + 1) * 128] for b in range(4)], axis=0).astype(BF)

            with scope("w_wuv"):
                wait_all(wuv_b, sems.at[3])
            with scope("c_wuv"):
                ctx = contract_lead(clat, wuv_b, lambda t: cache_step(kc_h, k_b, sems.at[5], t))
                for h in range(H):
                    cb_ref[h] = jnp.broadcast_to(ctx[h:h + 1, :], (8, DH))

            with scope("w_wq"):
                c_ax.wait()
                wait_all(wq_b, sems.at[4])
            with scope("c_wq"):
                xa = jnp.broadcast_to(ax_b[0].astype(F32), (8, DM)).astype(BF)

                def q_body(i, _):
                    qv = _dot(xa, wq_b[:, pl.ds(pl.multiple_of(i * 512, 512), 512)])
                    for u in range(4):
                        qa_ref[i * 4 + u] = qv[:, u * DH:(u + 1) * DH]
                stage(q_body, None, lambda t: cache_step(kc_h, k_b, sems.at[5], STEPS + t))
            stage(None, None, lambda t: cache_step(vc_h, v_b, sems.at[6], t))

            with scope("w_k"):
                wait_all(k_b, sems.at[5])
            with scope("c_k"):
                def k_body(t, _):
                    for i in range(4):
                        h = t * 4 + i
                        s = _dot_nt(qa_ref[h].astype(BF), k_b[h]) * scale
                        p = jnp.exp(s - jnp.max(s, axis=1, keepdims=True))
                        pa_ref[h] = p
                        la_ref[h] = jnp.broadcast_to(jnp.sum(p, axis=1, keepdims=True), (8, DH))
                stage(k_body, None, lambda t: cache_step(vc_h, v_b, sems.at[6], STEPS + t))
            stage(None, None, *row_stream(bwo_h, bwo_b, (sems.at[7], sems.at[10]), row_n, 8))
            wo_pairs(0, wo_early)

            with scope("w_v"):
                wait_all(v_b, sems.at[6])
            with scope("c_v"):
                def v_body(t, _):
                    for i in range(4):
                        h = t * 4 + i
                        oa_ref[h] = _dot(pa_ref[h].astype(BF), v_b[h]) / la_ref[h]
                stage(v_body, None, lambda t: None)
            wo_pairs(wo_early, len(wo_chunks))

            if not compute:
                wait_all(bwo_b.at[pl.ds(0, H * DH // 2)], sems.at[7])
                wait_all(bwo_b.at[pl.ds(H * DH // 2, H * DH // 2)], sems.at[10])
                for i in range(len(wo_chunks)):
                    wo_copy(i).wait()
                o_ref[...] = jnp.zeros(o_ref.shape, o_ref.dtype)
                return

            def bo_body(h, acc):
                return acc + _dot(cb_ref[h].astype(BF), bwo_b[pl.ds(pl.multiple_of(h * DH, DH), DH), :])
            ob = jnp.zeros((8, DM), F32)
            for u, sem in enumerate((sems.at[7], sems.at[10])):
                with scope("w_bwo"):
                    wait_all(bwo_b.at[pl.ds(u * (H * DH // 2), H * DH // 2)], sem)
                with scope("c_bwo"):
                    ob = lax.fori_loop(u * (H // 2), (u + 1) * (H // 2), bo_body, ob, unroll=8)
            o_ref[0, :, DM:2 * DM] = ob[0:1].astype(o_ref.dtype)

            waited = set()

            def wait_rows(r0, r1):
                for i in chunks_of(r0, r1):
                    if i not in waited:
                        waited.add(i)
                        wo_copy(i).wait()

            acc = jnp.zeros((8, DM), F32)
            with scope("wo_a"):
                pos = 0
                for bi in range(H):
                    heads = mxu_heads[pos:pos + batch[min(bi, len(batch) - 1)]]
                    pos += len(heads)
                    for h in heads:
                        wait_rows(h * DH, (h + 1) * DH)
                    for h in heads:
                        acc = acc + _dot(oa_ref[h].astype(BF), wo_b[h * DH:(h + 1) * DH, :])
                    if bi == 0:
                        for j in range(n_vpu):
                            o_h = oa_ref[H - n_vpu + j].astype(BF).astype(F32)
                            ot_ref[j * DH:(j + 1) * DH, :] = jnp.broadcast_to(o_h[0:1], (DH, DH)).T
            acc = jnp.where(lax.broadcasted_iota(jnp.int32, (8, DM), 0) == 0, acc, 0.0)
            r0 = vpu_start
            assert sum(vpu_groups) * 16 == n_vpu * DH
            for g in vpu_groups:
                wait_rows(r0, r0 + g * 16)
                for r in range(r0, r0 + g * 16, 8):
                    o_col = ot_ref[r - vpu_start:r - vpu_start + 8, :]
                    acc = acc + wo_b[r:r + 8, :].astype(F32) * jnp.concatenate([o_col] * (DM // DH), axis=1)
                r0 += g * 16
            assert len(waited) == len(wo_chunks)
            o_ref[0, :, 0:DM] = jnp.sum(acc, axis=0, keepdims=True).astype(o_ref.dtype)

        pl.run_scoped(main, pltpu.SemaphoreType.DMA((11,)), pltpu.SemaphoreType.DMA((len(wo_chunks),)))

    def fn(A_x, A_k_cache, A_v_cache, A_wq, A_wo, B_x, B_c_kv, B_w_q, B_w_uk, B_w_uv, B_w_o):
        sk = A_k_cache.shape[2]
        w = min(4096, max(256, sk // 4))
        skb = B_c_kv.shape[1]
        ck = skb // STEPS
        hbm = pl.BlockSpec(memory_space=pltpu.HBM)
        V = pltpu.VMEM
        return pl.pallas_call(
            kernel,
            out_shape=jax.ShapeDtypeStruct((1, 1, 2 * DM), BF),
            in_specs=[hbm] * 11,
            out_specs=pl.BlockSpec(memory_space=pltpu.VMEM),
            scratch_shapes=[
                V((1, 1, DM), BF), V((1, 1, DM), BF),
                V((H, w, DH), BF), V((H, w, DH), BF),
                V((DM, H * DH), BF), V((H * DH, DM), BF),
                V((skb, DM), BF), V((DM, H, DH), BF), V((DM, H, DH), BF), V((DM, H, DH), BF),
                V((H * DH, DM), BF),
                V((STEPS, H, ck), F32),
                V((H, 8, DH), F32), V((H, 8, w), F32), V((H, 8, DH), F32), V((H, 8, DH), F32),
                V((H, 8, DH), F32),
                V((n_vpu * DH, DH), F32),
            ],
            compiler_params=pltpu.CompilerParams(vmem_limit_bytes=64 * 1024 * 1024),
        )(A_x, A_k_cache, A_v_cache, A_wq, A_wo, B_x, B_c_kv, B_w_q, B_w_uk, B_w_uv, B_w_o.reshape(H * DH, DM))
    return fn


@jax.jit
def pallas_concat_heads__sliding_block_cached__compressed_kv_cla__decode_kernel(
    A_x, A_k_cache, A_v_cache, A_wq, A_wo, B_x, B_c_kv, B_w_q, B_w_uk, B_w_uv, B_w_o,
):
    return make(batch=(12, 8, 4, 3, 1, 1), n_vpu=3, vpu_groups=(8, 8, 4, 2, 1, 1))(
        A_x, A_k_cache, A_v_cache, A_wq, A_wo, B_x, B_c_kv, B_w_q, B_w_uk, B_w_uv, B_w_o)
```

```python
import contextlib
import jax
import jax.numpy as jnp
from jax import lax
from jax.experimental import pallas as pl
from jax.experimental.pallas import tpu as pltpu

BF = jnp.bfloat16
F32 = jnp.float32
H = 32
DH = 128
DM = 512
R = 4
NT = (((1,), (1,)), ((), ()))
STEPS = 8
PER = 8


def _dot(a, b):
    return jnp.dot(a, b, preferred_element_type=F32)


def _dot_nt(a, b):
    return lax.dot_general(a, b, NT, preferred_element_type=F32)


def _aligned(start, size, align):
    return pl.ds(start if isinstance(start, int) else pl.multiple_of(start, align), size)


def make(q=24, kv_heads=4, n_small=6, wo_early=12, vpu_groups=(8, 4, 2, 1, 1), compute=True, scopes=False):
    scope = (lambda n: jax.named_scope(n)) if scopes else (lambda n: contextlib.nullcontext())
    HR = H // R
    n_idx = HR * DH // 8
    wo_list = [(i, 0, R) for i in range(n_idx - n_small)] + [(i, a, 1) for i in range(n_idx - n_small, n_idx) for a in range(R)]
    n_lo = len(wo_list) // 2
    vpu_i0 = n_idx - DH // 8

    def kernel(ax_h, kc_h, vc_h, wq_h, wo_h, bx_h, ckv_h, bwq_h, wuk_h, wuv_h, bwo_h, o_ref,
               ax_b, bx_b, k_b, v_b, wq_b, wo_b, ckv_b, bwq_b, wuk_b, wuv_b, bwo_b,
               sb_ref, qa_ref, pa_ref, la_ref, oa_ref, cb_ref, ot_ref):
        sk = kc_h.shape[2]
        w = k_b.shape[1]
        scale = DH ** -0.5

        def main(sems, wo_sems):
            def lead_chunk(src, dst, sem):
                return lambda j: pltpu.make_async_copy(src.at[:, pl.ds(j, 1)], dst.at[:, pl.ds(j, 1)], sem)

            def row_chunk(src, dst, sem):
                def chunk(j):
                    r = _aligned(j * 8, 8, 8)
                    return pltpu.make_async_copy(src.at[:, r], dst.at[:, r], sem)
                return chunk

            def issue(lo, hi, t):
                for i in range(PER):
                    hi(STEPS * PER + t * PER + i).start(priority=1)
                    lo(t * PER + i).start(priority=0)

            def issue_wq(t):
                for i in range(PER):
                    for base, priority in ((STEPS, 1), (0, 0)):
                        r = _aligned((base + t) * 8, 8, 8)
                        c = pl.ds(i * 512, 512)
                        pltpu.make_async_copy(wq_h.at[:, r, c], wq_b.at[:, r, c], sems.at[4]).start(priority=priority)

            def issue_cache(src, dst, sem, t):
                n = 128 // kv_heads
                per_group = w // (n * PER)
                g = t // per_group
                k0 = (t - g * per_group) * (n * PER)
                for i in range(PER):
                    for base, priority in ((H // 2, 1), (0, 0)):
                        hs = pl.ds(base + g * kv_heads, kv_heads)
                        pltpu.make_async_copy(src.at[0, hs, _aligned(sk - w + k0 + i * n, n, n)],
                                              dst.at[hs, _aligned(k0 + i * n, n, n)], sem).start(priority=priority)

            def wo_sem(i):
                return wo_sems.at[i // 16] if i < vpu_i0 else wo_sems.at[HR - 1 + i - vpu_i0]

            def wo_pairs(j0, j1):
                for j in range(j0, j1):
                    for k, priority in ((n_lo + j, 1), (j, 0)):
                        if k < (len(wo_list) if priority else n_lo):
                            i, a, n = wo_list[k]
                            idx = (pl.ds(a, n), pl.ds(i * 8, 8))
                            pltpu.make_async_copy(wo_h.at[idx], wo_b.at[idx], wo_sem(i)).start(priority=priority)

            def wait_all(buf, sem):
                pltpu.make_async_copy(buf, buf, sem).wait()

            def stage(body, init, issue_fn):
                def step(t, carry):
                    issue_fn(t)
                    return body(t, carry) if compute and body is not None else carry
                return lax.fori_loop(0, STEPS, step, init)

            bwq_chunk = lead_chunk(bwq_h, bwq_b, sems.at[0])
            wuk_chunk = lead_chunk(wuk_h, wuk_b, sems.at[1])
            ckv_chunk = row_chunk(ckv_h, ckv_b, sems.at[2])
            wuv_chunk = lead_chunk(wuv_h, wuv_b, sems.at[3])
            c_bx = pltpu.make_async_copy(bx_h, bx_b, sems.at[9])
            c_ax = pltpu.make_async_copy(ax_h, ax_b, sems.at[10])

            n0 = (2 * STEPS * PER - q) // 2
            for j in range(n0 + q):
                bwq_chunk(n0 + j).start(priority=1)
                if j == 0:
                    c_bx.start()
                    c_ax.start()
                if j >= q:
                    bwq_chunk(j - q).start(priority=0)
            stage(None, None, lambda t: issue(wuk_chunk, wuk_chunk, t))

            row = lax.broadcasted_iota(jnp.int32, (128, 128), 0)
            lane = lax.broadcasted_iota(jnp.int32, (128, 128), 1)

            def diag_mask():
                return (row & (H - 1)) == (lane & (H - 1))

            def w_tile(ref, b, j):
                return ref[b, pl.ds(j * 4, 4)].reshape(128, 128)

            def contract_lead(a, w_ref, issue_fn):
                def body(t, acc):
                    for u in range(4):
                        j = t * 4 + u
                        et = (row - (lane >> 5) == 4 * j).astype(BF)
                        s = jnp.where(diag_mask(), _dot(a, et), 0.0).astype(BF)
                        for b in range(R):
                            acc = acc + _dot(s[b * H:(b + 1) * H], w_tile(w_ref, b, j))
                    return acc
                return stage(body, jnp.zeros((H, DH), F32), issue_fn)

            with scope("w_bwq"):
                c_bx.wait()
                wait_all(bwq_b, sems.at[0])
            with scope("c_bwq"):
                xb = bx_b[0].astype(F32)
                a = jnp.concatenate(
                    [jnp.broadcast_to(xb[:, b * 128:(b + 1) * 128], (H, 128)) for b in range(R)], axis=0).astype(BF)
                qb = contract_lead(a, bwq_b, lambda t: issue(ckv_chunk, ckv_chunk, t)).astype(BF)

            with scope("w_wuk"):
                wait_all(wuk_b, sems.at[1])
            with scope("c_wuk"):
                def uk_body(t, acc):
                    for u in range(4):
                        j = t * 4 + u
                        r = jnp.concatenate([_dot_nt(qb, w_tile(wuk_b, b, j)) for b in range(R)], axis=0)
                        r = jnp.where(diag_mask(), r, 0.0).astype(BF)
                        e = (lane - (row >> 5) == 4 * j).astype(BF)
                        acc = acc + _dot(r, e)
                    return acc
                qabs = stage(uk_body, jnp.zeros((128, 128), F32), lambda t: issue(wuv_chunk, wuv_chunk, t))
                qabs = jnp.concatenate([qabs[b * H:(b + 1) * H] for b in range(R)], axis=1).astype(BF)

            with scope("w_ckv"):
                wait_all(ckv_b, sems.at[2])
            with scope("c_ckv"):
                ck = sb_ref.shape[2]

                def keys(i):
                    return ckv_b[i // 2, _aligned((i % 2) * ck, ck, ck), :]

                def s_body(i, m):
                    s = _dot_nt(qabs, keys(i)) * scale
                    sb_ref[i] = s
                    return jnp.maximum(m, s)

                def half_issue(t0):
                    return lambda t: pl.when(t % 2 == 0)(lambda: issue_wq(t0 + t // 2))
                m = stage(s_body, jnp.full((H, ck), -jnp.inf, F32), half_issue(0))
                m = jnp.max(m, axis=1, keepdims=True)

                def pv_body(i, carry):
                    l, acc = carry
                    p = jnp.exp(sb_ref[i] - m)
                    return l + p, acc + _dot(p.astype(BF), keys(i))
                l, clat = stage(pv_body, (jnp.zeros((H, ck), F32), jnp.zeros((H, DM), F32)), half_issue(STEPS // 2))
                clat = clat / jnp.sum(l, axis=1, keepdims=True)
                clat = jnp.concatenate([clat[:, b * 128:(b + 1) * 128] for b in range(R)], axis=0).astype(BF)

            with scope("w_wuv"):
                wait_all(wuv_b, sems.at[3])
            with scope("c_wuv"):
                ctx = contract_lead(clat, wuv_b, lambda t: issue_cache(kc_h, k_b, sems.at[5], t))
                for h in range(H):
                    cb_ref[h] = jnp.broadcast_to(ctx[h:h + 1, :], (8, DH))

            with scope("w_wq"):
                c_ax.wait()
                wait_all(wq_b, sems.at[4])
            with scope("c_wq"):
                xa = jnp.broadcast_to(ax_b[0].astype(F32), (8, DM)).astype(BF)

                def q_body(i, _):
                    cols = _aligned(i * 512, 512, 512)
                    qv = _dot(xa[:, 0:128], wq_b[0, :, cols])
                    for b in range(1, R):
                        qv = qv + _dot(xa[:, b * 128:(b + 1) * 128], wq_b[b, :, cols])
                    for u in range(4):
                        qa_ref[i * 4 + u] = qv[:, u * DH:(u + 1) * DH]
                stage(q_body, None, lambda t: issue_cache(kc_h, k_b, sems.at[5], STEPS + t))
            stage(None, None, lambda t: issue_cache(vc_h, v_b, sems.at[6], t))

            with scope("w_k"):
                wait_all(k_b, sems.at[5])
            with scope("c_k"):
                def k_body(t, _):
                    for i in range(4):
                        h = t * 4 + i
                        s = _dot_nt(qa_ref[h].astype(BF), k_b[h]) * scale
                        p = jnp.exp(s - jnp.max(s, axis=1, keepdims=True))
                        pa_ref[h] = p
                        la_ref[h] = jnp.broadcast_to(jnp.sum(p, axis=1, keepdims=True), (8, DH))
                stage(k_body, None, lambda t: issue_cache(vc_h, v_b, sems.at[6], STEPS + t))
            stage(None, None, lambda t: issue(row_chunk(bwo_h, bwo_b, sems.at[7]), row_chunk(bwo_h, bwo_b, sems.at[8]), t))
            wo_pairs(0, wo_early)

            with scope("w_v"):
                wait_all(v_b, sems.at[6])
            n_mid = (len(wo_list) - n_lo + wo_early) // 2
            for u in range(2):
                with scope("c_v"):
                    def v_body(t, _):
                        for i in range(4):
                            h = t * 4 + i
                            oa_ref[h] = _dot(pa_ref[h].astype(BF), v_b[h]) / la_ref[h]
                    if compute:
                        lax.fori_loop(u * STEPS // 2, (u + 1) * STEPS // 2, v_body, None)
                wo_pairs(*((wo_early, n_mid), (n_mid, len(wo_list)))[u])

            half = HR * DH // 2
            if not compute:
                wait_all(bwo_b.at[:, pl.ds(0, half)], sems.at[7])
                wait_all(bwo_b.at[:, pl.ds(half, half)], sems.at[8])
                for g in range(HR - 1):
                    wait_all(wo_b.at[:, pl.ds(g * DH, DH)], wo_sems.at[g])
                for i in range(vpu_i0, n_idx):
                    wait_all(wo_b.at[:, pl.ds(i * 8, 8)], wo_sem(i))
                o_ref[...] = jnp.zeros(o_ref.shape, o_ref.dtype)
                return

            def project(acc, c_ref, w_ref, g):
                for a in range(R):
                    acc = acc + _dot(c_ref[a * HR + g].astype(BF), w_ref[a, _aligned(g * DH, DH, DH), :])
                return acc

            ob = jnp.zeros((8, DM), F32)
            for u in range(2):
                with scope("w_bwo"):
                    wait_all(bwo_b.at[:, pl.ds(u * half, half)], sems.at[7 + u])
                with scope("c_bwo"):
                    ob = lax.fori_loop(u * HR // 2, (u + 1) * HR // 2,
                                       lambda g, acc: project(acc, cb_ref, bwo_b, g), ob, unroll=2)
            o_ref[0, :, DM:2 * DM] = ob[0:1].astype(o_ref.dtype)

            for a in range(R):
                o_h = oa_ref[a * HR + HR - 1].astype(BF).astype(F32)
                ot_ref[a] = jnp.broadcast_to(o_h[0:1], (DH, DH)).T

            arrival = lambda k: k if k < n_lo else k - n_lo + q
            acc = jnp.zeros((8, DM), F32)
            with scope("wo_a"):
                for g in sorted(range(HR - 1), key=lambda g: max(arrival(k) for k in range(g * 16, g * 16 + 16))):
                    wait_all(wo_b.at[:, pl.ds(g * DH, DH)], wo_sems.at[g])
                    acc = project(acc, oa_ref, wo_b, g)
            acc = jnp.where(lax.broadcasted_iota(jnp.int32, (8, DM), 0) == 0, acc, 0.0)
            i0 = vpu_i0
            for n in vpu_groups:
                for i in range(i0, i0 + n):
                    wait_all(wo_b.at[:, pl.ds(i * 8, 8)], wo_sem(i))
                for i in range(i0, i0 + n):
                    for a in range(R):
                        o_col = ot_ref[a, (i - vpu_i0) * 8:(i - vpu_i0) * 8 + 8, :]
                        acc = acc + wo_b[a, i * 8:i * 8 + 8, :].astype(F32) * jnp.concatenate([o_col] * (DM // DH), axis=1)
                i0 += n
            assert i0 == n_idx
            o_ref[0, :, 0:DM] = jnp.sum(acc, axis=0, keepdims=True).astype(o_ref.dtype)

        pl.run_scoped(main, pltpu.SemaphoreType.DMA((11,)), pltpu.SemaphoreType.DMA((HR - 1 + n_idx - vpu_i0,)))

    def fn(A_x, A_k_cache, A_v_cache, A_wq, A_wo, B_x, B_c_kv, B_w_q, B_w_uk, B_w_uv, B_w_o):
        sk = A_k_cache.shape[2]
        w = min(4096, max(256, sk // 4))
        skb = B_c_kv.shape[1]
        hbm = pl.BlockSpec(memory_space=pltpu.HBM)
        V = pltpu.VMEM
        lead = (R, DM // R, H, DH)
        rows = (R, H * DH // R, DM)
        wq_shape = (R, DM // R, H * DH)
        return pl.pallas_call(
            kernel,
            out_shape=jax.ShapeDtypeStruct((1, 1, 2 * DM), BF),
            in_specs=[hbm] * 11,
            out_specs=pl.BlockSpec(memory_space=pltpu.VMEM),
            scratch_shapes=[
                V((1, 1, DM), BF), V((1, 1, DM), BF),
                V((H, w, DH), BF), V((H, w, DH), BF),
                V(wq_shape, BF), V(rows, BF),
                V(rows, BF), V(lead, BF), V(lead, BF), V(lead, BF),
                V(rows, BF),
                V((STEPS, H, skb // STEPS), F32),
                V((H, 8, DH), F32), V((H, 8, w), F32), V((H, 8, DH), F32), V((H, 8, DH), F32),
                V((H, 8, DH), F32),
                V((R, DH, DH), F32),
            ],
            compiler_params=pltpu.CompilerParams(vmem_limit_bytes=64 * 1024 * 1024),
        )(A_x, A_k_cache, A_v_cache, A_wq.reshape(wq_shape), A_wo.reshape(rows), B_x, B_c_kv.reshape(rows),
          B_w_q.reshape(lead), B_w_uk.reshape(lead), B_w_uv.reshape(lead), B_w_o.reshape(rows))
    return fn


@jax.jit
def pallas_concat_heads__sliding_block_cached__compressed_kv_cla__decode_kernel(
    A_x, A_k_cache, A_v_cache, A_wq, A_wo, B_x, B_c_kv, B_w_q, B_w_uk, B_w_uv, B_w_o,
):
    return make(n_small=0)(
        A_x, A_k_cache, A_v_cache, A_wq, A_wo, B_x, B_c_kv, B_w_q, B_w_uk, B_w_uv, B_w_o)
```

```python
import functools

import jax
import jax.numpy as jnp
from jax import lax
from jax.experimental import pallas as pl
from jax.experimental.pallas import tpu as pltpu

BF16 = jnp.bfloat16
F32 = jnp.float32

H = 32
DH = 128
DM = 512
R = 4
HR = H // R

STEPS = 8
PER = 8
HALF = STEPS * PER
PREFILL = 26
SHIFT = 27
KV_HEADS = 8
TAIL_GROUPS = (6, 4, 2, 2, 1, 1)


def _dot(a, b):
    return jnp.dot(a, b, preferred_element_type=F32)


def _dot_nt(a, b):
    return lax.dot_general(a, b, (((1,), (1,)), ((), ())), preferred_element_type=F32)


def _tile(i, size):
    start = i * size
    return pl.ds(start if isinstance(start, int) else pl.multiple_of(start, size), size)


def _copy(src, dst, idx, sem):
    return pltpu.make_async_copy(src.at[idx], dst.at[idx], sem)


def _wait_all(buf, sem):
    pltpu.make_async_copy(buf, buf, sem).wait()


def _stage(issue, fn=None, init=None):
    def step(t, carry):
        issue(t)
        return carry if fn is None else fn(t, carry)
    return lax.fori_loop(0, STEPS, step, init)


def _body(ax_hbm, kc_hbm, vc_hbm, wq_hbm, wo_hbm, bx_hbm, ckv_hbm, bwq_hbm, wuk_hbm, wuv_hbm, bwo_hbm,
          out_ref,
          ax, bx, keys_a, values_a, wq, wo, ckv, bwq, wuk, wuv, bwo,
          scores_b, q_a, p_a, l_a, ctx_a, ctx_b, ctx_cols,
          sems, wo_sems):
    sk, window = kc_hbm.shape[2], keys_a.shape[1]
    scale = DH ** -0.5
    names = ("ax", "bx", "bwq", "wuk", "ckv", "wuv", "wq", "k", "v", "bwo_lo", "bwo_hi")
    sem = {name: sems.at[i] for i, name in enumerate(names)}
    every = slice(None)

    def lead_piece(src, dst, s):
        return lambda j: _copy(src, dst, (every, pl.ds(j, 1)), s)

    def row_piece(src, dst, s):
        return lambda j: _copy(src, dst, (every, _tile(j, 8)), s)

    def wq_piece(j):
        return _copy(wq_hbm, wq, (every, _tile(j >> 3, 8), _tile(j & 7, 512)), sem["wq"])

    def unit(lo, hi=None):
        def issue(t):
            for i in range(PER):
                j = t * PER + i
                (hi or lo)(HALF + j).start(priority=1)
                lo((j - SHIFT) & (HALF - 1)).start(priority=0)
        return issue

    def cache_unit(src, dst, s, part):
        n = 128 // KV_HEADS
        group_steps = window // (n * PER)
        first = (sk - window) // n

        def issue(t):
            t = part * STEPS + t
            for i in range(PER):
                for h0, tt, priority in ((H // 2, t, 1), (0, (t - SHIFT // PER) & (2 * STEPS - 1), 0)):
                    g = tt // group_steps
                    k = (tt - g * group_steps) * PER + i
                    heads = pl.ds(h0 + g * KV_HEADS, KV_HEADS)
                    pltpu.make_async_copy(src.at[0, heads, _tile(first + k, n)],
                                          dst.at[heads, _tile(k, n)], s).start(priority=priority)
        return issue

    tail_start = 2 * HALF - DH // 8

    def wo_sem(i):
        return wo_sems.at[i // (DH // 8)] if i < tail_start else wo_sems.at[HR - 1 + i - tail_start]

    def issue_wo(j0, j1):
        for j in range(j0, j1):
            for i, priority in ((HALF + j, 1), ((j - SHIFT) % HALF, 0)):
                _copy(wo_hbm, wo, (every, _tile(i, 8)), wo_sem(i)).start(priority=priority)

    copy_ax = pltpu.make_async_copy(ax_hbm, ax, sem["ax"])
    copy_bx = pltpu.make_async_copy(bx_hbm, bx, sem["bx"])
    bwq_piece = lead_piece(bwq_hbm, bwq, sem["bwq"])
    n_lo = HALF - PREFILL // 2
    for j in range(n_lo + PREFILL):
        bwq_piece(n_lo + j).start(priority=1)
        if j == 0:
            copy_bx.start()
            copy_ax.start()
        if j >= PREFILL:
            bwq_piece(j - PREFILL).start(priority=0)
    _stage(unit(lead_piece(wuk_hbm, wuk, sem["wuk"])))

    row = lax.broadcasted_iota(jnp.int32, (128, 128), 0)
    lane = lax.broadcasted_iota(jnp.int32, (128, 128), 1)

    def same_head():
        return (row & (H - 1)) == (lane & (H - 1))

    def w_tile(ref, b, j):
        return ref[b, pl.ds(j * 4, 4)].reshape(128, 128)

    def contract_c(a, w_ref, issue):
        def fn(t, acc):
            for u in range(4):
                j = t * 4 + u
                spread = (row - (lane >> 5) == 4 * j).astype(BF16)
                s = jnp.where(same_head(), _dot(a, spread), 0.0).astype(BF16)
                for b in range(R):
                    acc = acc + _dot(s[b * H:(b + 1) * H], w_tile(w_ref, b, j))
            return acc
        return _stage(issue, fn, jnp.zeros((H, DH), F32))

    def contract_d(q, w_ref, issue):
        def fn(t, acc):
            for u in range(4):
                j = t * 4 + u
                r = jnp.concatenate([_dot_nt(q, w_tile(w_ref, b, j)) for b in range(R)], axis=0)
                r = jnp.where(same_head(), r, 0.0).astype(BF16)
                gather = (lane - (row >> 5) == 4 * j).astype(BF16)
                acc = acc + _dot(r, gather)
            return acc
        return _stage(issue, fn, jnp.zeros((R * H, 128), F32))

    copy_bx.wait()
    _wait_all(bwq, sem["bwq"])
    x_b = bx[0].astype(F32)
    x_b = jnp.concatenate(
        [jnp.broadcast_to(x_b[:, b * 128:(b + 1) * 128], (H, 128)) for b in range(R)], axis=0).astype(BF16)
    q_b = contract_c(x_b, bwq, unit(row_piece(ckv_hbm, ckv, sem["ckv"]))).astype(BF16)

    _wait_all(wuk, sem["wuk"])
    q_lat = contract_d(q_b, wuk, unit(lead_piece(wuv_hbm, wuv, sem["wuv"])))
    q_lat = jnp.concatenate([q_lat[b * H:(b + 1) * H] for b in range(R)], axis=1).astype(BF16)

    _wait_all(ckv, sem["ckv"])
    block = scores_b.shape[2]

    def latent(t):
        return ckv[t >> 1, _tile(t & 1, block), :]

    def half_rate(t0):
        return lambda t: pl.when((t & 1) == 0)(lambda: unit(wq_piece)(t0 + (t >> 1)))

    def score_fn(t, m):
        s = _dot_nt(q_lat, latent(t)) * scale
        scores_b[t] = s
        return jnp.maximum(m, s)
    m_b = _stage(half_rate(0), score_fn, jnp.full((H, block), -jnp.inf, F32))
    m_b = jnp.max(m_b, axis=1, keepdims=True)

    def mix_fn(t, carry):
        l, acc = carry
        p = jnp.exp(scores_b[t] - m_b)
        return l + p, acc + _dot(p.astype(BF16), latent(t))
    l_b, ctx_lat = _stage(half_rate(STEPS // 2), mix_fn, (jnp.zeros((H, block), F32), jnp.zeros((H, DM), F32)))
    ctx_lat = ctx_lat / jnp.sum(l_b, axis=1, keepdims=True)
    ctx_lat = jnp.concatenate([ctx_lat[:, b * 128:(b + 1) * 128] for b in range(R)], axis=0).astype(BF16)

    _wait_all(wuv, sem["wuv"])
    ctx = contract_c(ctx_lat, wuv, cache_unit(kc_hbm, keys_a, sem["k"], 0))
    for h in range(H):
        ctx_b[h] = jnp.broadcast_to(ctx[h:h + 1, :], (8, DH))

    copy_ax.wait()
    _wait_all(wq, sem["wq"])
    x_a = jnp.broadcast_to(ax[0].astype(F32), (8, DM)).astype(BF16)

    def query_fn(t, _):
        cols = _tile(t, 4 * DH)
        q = _dot(x_a[:, 0:128], wq[0, :, cols])
        for b in range(1, R):
            q = q + _dot(x_a[:, b * 128:(b + 1) * 128], wq[b, :, cols])
        for i in range(4):
            q_a[t * 4 + i] = q[:, i * DH:(i + 1) * DH]
    _stage(cache_unit(kc_hbm, keys_a, sem["k"], 1), query_fn)
    _stage(cache_unit(vc_hbm, values_a, sem["v"], 0))

    _wait_all(keys_a, sem["k"])

    def softmax_fn(t, _):
        for i in range(4):
            h = t * 4 + i
            s = _dot_nt(q_a[h].astype(BF16), keys_a[h]) * scale
            p = jnp.exp(s - jnp.max(s, axis=1, keepdims=True))
            p_a[h] = p
            l_a[h] = jnp.broadcast_to(jnp.sum(p, axis=1, keepdims=True), (8, DH))
    _stage(cache_unit(vc_hbm, values_a, sem["v"], 1), softmax_fn)
    _stage(unit(row_piece(bwo_hbm, bwo, sem["bwo_lo"]), row_piece(bwo_hbm, bwo, sem["bwo_hi"])))

    issue_wo(0, 12)
    _wait_all(values_a, sem["v"])

    def context_fn(h, _):
        ctx_a[h] = _dot(p_a[h].astype(BF16), values_a[h]) / l_a[h]
    lax.fori_loop(0, H // 2, context_fn, None, unroll=4)
    issue_wo(12, 38)
    lax.fori_loop(H // 2, H, context_fn, None, unroll=4)
    issue_wo(38, HALF)

    def project(acc, ctx_ref, w_ref, g):
        for a in range(R):
            acc = acc + _dot(ctx_ref[a * HR + g].astype(BF16), w_ref[a, _tile(g, DH), :])
        return acc

    out_b = jnp.zeros((8, DM), F32)
    for u, name in enumerate(("bwo_lo", "bwo_hi")):
        _wait_all(bwo.at[:, _tile(u, HR * DH // 2)], sem[name])
        out_b = lax.fori_loop(u * HR // 2, (u + 1) * HR // 2,
                              lambda g, acc: project(acc, ctx_b, bwo, g), out_b, unroll=2)
    out_ref[0, :, DM:2 * DM] = out_b[0:1].astype(out_ref.dtype)

    for a in range(R):
        last = ctx_a[a * HR + HR - 1].astype(BF16).astype(F32)
        ctx_cols[a] = jnp.broadcast_to(last[0:1], (DH, DH)).T

    def arrival(g):
        pieces = range(g * DH // 8, (g + 1) * DH // 8)
        return max((i + SHIFT) % HALF if i < HALF else i - HALF + PREFILL for i in pieces)

    out_a = jnp.zeros((8, DM), F32)
    for g in sorted(range(HR - 1), key=arrival):
        _wait_all(wo.at[:, _tile(g, DH)], wo_sems.at[g])
        out_a = project(out_a, ctx_a, wo, g)
    out_a = jnp.where(lax.broadcasted_iota(jnp.int32, (8, DM), 0) == 0, out_a, 0.0)
    i0 = tail_start
    for n in TAIL_GROUPS:
        for i in range(i0, i0 + n):
            _wait_all(wo.at[:, _tile(i, 8)], wo_sem(i))
        for i in range(i0, i0 + n):
            for a in range(R):
                col = ctx_cols[a, _tile(i - tail_start, 8), :]
                out_a = out_a + wo[a, _tile(i, 8), :].astype(F32) * jnp.concatenate([col] * (DM // DH), axis=1)
        i0 += n
    assert i0 == 2 * HALF
    out_ref[0, :, 0:DM] = jnp.sum(out_a, axis=0, keepdims=True).astype(out_ref.dtype)


def _kernel(*refs):
    pl.run_scoped(functools.partial(_body, *refs),
                  pltpu.SemaphoreType.DMA((11,)),
                  pltpu.SemaphoreType.DMA((HR - 1 + DH // 8,)))


@jax.jit
def pallas_concat_heads__sliding_block_cached__compressed_kv_cla__decode_kernel(
    A_x: jax.Array,
    A_k_cache: jax.Array,
    A_v_cache: jax.Array,
    A_wq: jax.Array,
    A_wo: jax.Array,
    B_x: jax.Array,
    B_c_kv: jax.Array,
    B_w_q: jax.Array,
    B_w_uk: jax.Array,
    B_w_uv: jax.Array,
    B_w_o: jax.Array,
):
    window = min(4096, max(256, A_k_cache.shape[2] // 4))
    assert A_x.shape == B_x.shape == (1, 1, DM)
    assert A_k_cache.shape == A_v_cache.shape == (1, H, 4 * window, DH) and window == 2 * STEPS * PER * 8
    assert B_c_kv.shape == (1, H * DH, DM) and B_w_q.shape == B_w_uk.shape == B_w_uv.shape == (DM, H, DH)

    lead = (R, DM // R, H, DH)
    rows = (R, H * DH // R, DM)
    cols = (R, DM // R, H * DH)
    vmem = pltpu.VMEM
    per_head = vmem((H, 8, DH), F32)
    return pl.pallas_call(
        _kernel,
        out_shape=jax.ShapeDtypeStruct((1, 1, 2 * DM), BF16),
        in_specs=[pl.BlockSpec(memory_space=pltpu.HBM)] * 11,
        out_specs=pl.BlockSpec(memory_space=pltpu.VMEM),
        scratch_shapes=[
            vmem((1, 1, DM), BF16), vmem((1, 1, DM), BF16),
            vmem((H, window, DH), BF16), vmem((H, window, DH), BF16),
            vmem(cols, BF16), vmem(rows, BF16),
            vmem(rows, BF16), vmem(lead, BF16), vmem(lead, BF16), vmem(lead, BF16),
            vmem(rows, BF16),
            vmem((STEPS, H, B_c_kv.shape[1] // STEPS), F32),
            per_head, vmem((H, 8, window), F32), per_head,
            per_head, per_head, vmem((R, DH, DH), F32),
        ],
        compiler_params=pltpu.CompilerParams(vmem_limit_bytes=64 * 1024 * 1024),
    )(A_x, A_k_cache, A_v_cache, A_wq.reshape(cols), A_wo.reshape(rows), B_x, B_c_kv.reshape(rows),
      B_w_q.reshape(lead), B_w_uk.reshape(lead), B_w_uv.reshape(lead), B_w_o.reshape(rows))
```
